```python
import os as _os
_os.environ.setdefault("JAX_PLATFORMS", "cpu")
import jax
import jax.numpy as jnp

def _softmax(x, axis=-1):
    return jax.nn.softmax(x, axis=axis)
def _gelu(x):
    return jax.nn.gelu(x, approximate=True)
def _silu(x):
    return jax.nn.silu(x)
def _sigmoid(x):
    return jax.nn.sigmoid(x)
def _layernorm(x, axis=-1, eps=1e-5):
    m = jnp.mean(x, axis=axis, keepdims=True)
    v = jnp.var(x, axis=axis, keepdims=True)
    return (x - m) / jnp.sqrt(v + eps)
def _scatter_add(tgt, idx, src, axis=0):
    return tgt.at[idx].add(src)
def _segment_sum(src, seg, n):
    return jax.ops.segment_sum(src, seg, n)
class _Rng:
    def __init__(self, key):
        self._k = key
    def _next(self):
        self._k, sub = jax.random.split(self._k)
        return sub
    def normal(self, shape):
        return jax.random.normal(self._next(), shape, dtype=jnp.bfloat16)
    def randint(self, lo, hi, shape):
        return jax.random.randint(self._next(), shape, lo, hi, dtype=jnp.int32)
    def uniform(self, shape, lo=0.0, hi=1.0):
        return jax.random.uniform(self._next(), shape, jnp.bfloat16, lo, hi)
    def permutation(self, n):
        return jax.random.permutation(self._next(), n)


kernel_name = 'sequential_preLN__sliding_block__mixer_channel_mlp__prompt'

def setup_inputs():
    _rng = _Rng(jax.random.key(int.from_bytes(__import__("os").urandom(4), "little")))
    _w = (lambda a: (lambda t: t.astype(jnp.bfloat16) if jnp.issubdtype(t.dtype, jnp.floating) else t)(jnp.asarray(a)))
    def _A_setup():
        B, S, D = 1, 2048, 1024
        return {
            "x": _w((lambda *s: _rng.normal(s) * 0.05)(B, S, D)),
            "wqkv": _w((lambda *s: _rng.normal(s) * 0.05)(D, 3 * D)),
            "wo": _w((lambda *s: _rng.normal(s) * 0.05)(D, D)),
        }
    _A_in = _A_setup()

    def _B_setup():
        B, S, D, F = 1, 2048, 1024, 3584
        return {
            "x": _w((lambda *s: _rng.normal(s) * 0.05)(B, S, D)),
            "w1": _w((lambda *s: _rng.normal(s) * 0.8)(D, F) * (D ** -0.5)),
            "b1": _w((lambda *s: _rng.normal(s) * 0.8)(F)),
            "w2": _w((lambda *s: _rng.normal(s) * 0.8)(F, D) * (F ** -0.5)),
            "b2": _w((lambda *s: _rng.normal(s) * 0.05)(D)),
        }
    _B_in = _B_setup()

    return {
        "A_x": _A_in["x"],
        "A_wqkv": _A_in["wqkv"],
        "A_wo": _A_in["wo"],
        "B_x": _B_in["x"],
        "B_w1": _B_in["w1"],
        "B_b1": _B_in["b1"],
        "B_w2": _B_in["w2"],
        "B_b2": _B_in["b2"],
    }

def reference(A_x, A_wqkv, A_wo, B_x, B_w1, B_b1, B_w2, B_b2):
    def _A_ref(x, wqkv, wo):
        B, S, D = x.shape
        H = 32; Dh = D // H; W = 256
        qkv = (lambda x, *d: x.transpose(*d))((x @ wqkv).reshape(B, S, 3, H, Dh), 2, 0, 3, 1, 4)
        q, k, v = qkv[0], qkv[1], qkv[2]
        scores = jnp.einsum("bhqd,bhkd->bhqk", q, k) * (Dh ** -0.5)
        idx = jnp.arange(S)
        mask = (idx[:, None] - idx[None, :] >= 0) & (idx[:, None] - idx[None, :] < W)
        scores = jnp.where(mask[None, None], scores, -1e9)
        p = _softmax(scores, axis=-1)
        o = jnp.einsum("bhqk,bhkd->bhqd", p, v)
        return (lambda x, *d: x.transpose(*d))(o, 0, 2, 1, 3).reshape(B, S, D) @ wo

    def _B_ref(x, w1, b1, w2, b2):
        y = _layernorm(x, axis=-1)
        h = _gelu(jnp.einsum("bsd,df->bsf", y, w1) + b1)
        return jnp.einsum("bsf,fd->bsd", h, w2) + b2

    x = A_x
    h = x + _A_ref(_layernorm(x, axis=-1), A_wqkv, A_wo)
    h2 = h + _B_ref(_layernorm(h, axis=-1), B_w1, B_b1, B_w2, B_b2)
    return h2
```

```python
import functools

import jax
import jax.numpy as jnp
import jax.experimental.pallas as pl
import jax.experimental.pallas.tpu as pltpu

S = 2048
D = 1024
H = 32
DH = 32
W = 256
F = 3584
HG = 8
QB = 128
TM = 128
NQB = TM // QB
NS = S // TM
SKEW = 3
NSLOT = SKEW + 1
EPS = 1e-5
NEG = -1e30
QSCALE = (DH ** -0.5) * 1.4426950408889634
FC = 256
NC = 128
NF = F // FC
NN = D // NC
ORDER = 'D'
ATT = 2


def _layernorm(x):
    m = jnp.mean(x, axis=-1, keepdims=True)
    xc = x - m
    v = jnp.mean(xc * xc, axis=-1, keepdims=True)
    return xc * jax.lax.rsqrt(v + EPS)


def _gelu_tanh(x):
    c = 0.7978845608028654
    inner = x * (c + (c * 0.044715) * (x * x))
    hx = 0.5 * x
    return hx + hx * jnp.tanh(inner)


def _dot(a, b):
    return jnp.dot(a, b, preferred_element_type=jnp.float32)


def _kernel(x_ref, wqkv_hbm, wo_hbm, w1_hbm, b1_ref, w2_hbm, b2_ref, o_ref,
            wqkv_v, wo_v, w1_v, w2_v, k_scr, vt_scr, qm_scr, ot_scr, y_scr, h_scr, hh_scr, s_scr, p_scr, sems):
    step = pl.program_id(0)
    fslot = step % NSLOT
    bslot = (step + 1) % NSLOT

    copies = [
        pltpu.make_async_copy(wqkv_hbm.at[:, 0:D], wqkv_v.at[:, 0:D], sems.at[0]),
        pltpu.make_async_copy(wqkv_hbm.at[:, D:2 * D], wqkv_v.at[:, D:2 * D], sems.at[1]),
        pltpu.make_async_copy(wqkv_hbm.at[:, 2 * D:3 * D], wqkv_v.at[:, 2 * D:3 * D], sems.at[2]),
        pltpu.make_async_copy(wo_hbm, wo_v, sems.at[3]),
        pltpu.make_async_copy(w1_hbm, w1_v, sems.at[4]),
        pltpu.make_async_copy(w2_hbm, w2_v, sems.at[5]),
    ]

    def wait_first(i):
        @pl.when(step == 0)
        def _():
            copies[i].wait()

    def make_front(first):
        st = {}

        def f_ln1():
            x = x_ref[...].astype(jnp.float32)
            st["xn"] = _layernorm(x).astype(jnp.bfloat16)

        def f_q():
            if first:
                wait_first(0)
            q = _dot(st["xn"], wqkv_v[:, 0:D]) * QSCALE
            lane = jax.lax.broadcasted_iota(jnp.int32, (TM, 128), 1)
            for hg in range(HG):
                qh = q[:, 128 * hg:128 * (hg + 1)]
                for g in range(4):
                    qm_scr[hg, g] = jnp.where((lane >= 32 * g) & (lane < 32 * (g + 1)), qh, 0.0).astype(jnp.bfloat16)

        def f_k():
            if first:
                wait_first(1)
            row0 = pl.multiple_of(step * TM, TM)
            k = _dot(st["xn"], wqkv_v[:, D:2 * D]).astype(jnp.bfloat16)
            for hg in range(HG):
                k_scr[hg, pl.ds(row0 + W, TM), :] = k[:, 128 * hg:128 * (hg + 1)]

        def f_v():
            if first:
                wait_first(2)
            v = _dot(st.pop("xn"), wqkv_v[:, 2 * D:3 * D])
            for t in range(NQB):
                vt_scr[step * NQB + 2 + t] = v[QB * t:QB * (t + 1), :].T.astype(jnp.bfloat16)

        def qk(s):
            lqb, hg = divmod(s, HG)
            par = s % 2
            gq0 = pl.multiple_of((step * NQB + lqb) * QB, QB)
            gqb = step * NQB + lqb
            qm = qm_scr[hg, :, QB * lqb:QB * (lqb + 1), :].reshape(4 * QB, 128)
            kp = k_scr[hg, pl.ds(gq0, 3 * QB), :]
            if ATT >= 1:
                kp = jnp.concatenate(
                    [x for r in range(8) for x in (kp[16 * r:16 * r + 16], kp[256 + 16 * r:256 + 16 * r + 16])]
                    + [kp[128:256]], axis=0)
            sT = jax.lax.dot_general(kp, qm, (((1,), (1,)), ((), ())),
                                     preferred_element_type=jnp.float32)
            lane = jax.lax.broadcasted_iota(jnp.int32, (QB, QB), 1)
            row = jax.lax.broadcasted_iota(jnp.int32, (QB, QB), 0)
            tri = jnp.concatenate([lane < row] * 4, axis=1)
            if ATT >= 1:
                s0 = jnp.concatenate([sT[32 * r:32 * r + 16] for r in range(8)], axis=0)
                s2 = jnp.concatenate([sT[32 * r + 16:32 * r + 32] for r in range(8)], axis=0)
                s1 = sT[256:384]
            else:
                s0, s1, s2 = sT[0:QB], sT[QB:2 * QB], sT[2 * QB:3 * QB]
            if first:
                s0 = jnp.where(gqb >= 2, s0, NEG)
                s1 = jnp.where(gqb >= 1, s1, NEG)
            sm_ = jnp.where(tri, s0, s2)
            m = jnp.maximum(jnp.max(sm_, axis=0, keepdims=True), jnp.max(s1, axis=0, keepdims=True))
            if ATT >= 2:
                s_scr[par, 0:QB, :] = sm_
                s_scr[par, QB:2 * QB, :] = s1
                st["m", s] = m
            else:
                st["m", s] = (m, sm_, s1)

        def sm(s):
            par = s % 2
            lane = jax.lax.broadcasted_iota(jnp.int32, (QB, QB), 1)
            row = jax.lax.broadcasted_iota(jnp.int32, (QB, QB), 0)
            tri = jnp.concatenate([lane < row] * 4, axis=1)
            if ATT >= 2:
                m = st.pop(("m", s))
                sm_ = s_scr[par, 0:QB, :]
                s1 = s_scr[par, QB:2 * QB, :]
            else:
                m, sm_, s1 = st.pop(("m", s))
            pm = jnp.exp2(sm_ - m)
            p1 = jnp.exp2(s1 - m)
            l = jnp.sum(pm, axis=0, keepdims=True) + jnp.sum(p1, axis=0, keepdims=True)
            tri1 = lane < row
            if ATT >= 3:
                p_scr[par, 0:QB, :] = jnp.where(tri, pm, 0.0).astype(jnp.bfloat16)
                p_scr[par, QB:2 * QB, :] = p1.astype(jnp.bfloat16)
                p_scr[par, 2 * QB:3 * QB, :] = jnp.where(tri, 0.0, pm).astype(jnp.bfloat16)
                st["p", s] = l
            else:
                ps = []
                for g in range(4):
                    gs = slice(QB * g, QB * (g + 1))
                    ps.append((jnp.where(tri1, pm[:, gs], 0.0).astype(jnp.bfloat16),
                               p1[:, gs].astype(jnp.bfloat16),
                               jnp.where(tri1, 0.0, pm[:, gs]).astype(jnp.bfloat16)))
                st["p", s] = (ps, l)

        def pv(s):
            lqb, hg = divmod(s, HG)
            par = s % 2
            gqb = step * NQB + lqb
            if ATT >= 3:
                l = st.pop(("p", s))
            else:
                ps, l = st.pop(("p", s))
            for g in range(4):
                gs = slice(QB * g, QB * (g + 1))
                r0 = (hg * 4 + g) * DH
                if ATT >= 3:
                    a0, a1, a2 = p_scr[par, 0:QB, gs], p_scr[par, QB:2 * QB, gs], p_scr[par, 2 * QB:3 * QB, gs]
                else:
                    a0, a1, a2 = ps[g]
                ot = (_dot(vt_scr[gqb, r0:r0 + DH, :], a0)
                      + _dot(vt_scr[gqb + 1, r0:r0 + DH, :], a1)
                      + _dot(vt_scr[gqb + 2, r0:r0 + DH, :], a2))
                ot_scr[lqb, r0:r0 + DH, :] = (ot / l[:, gs]).astype(ot_scr.dtype)

        def f_wo():
            if first:
                wait_first(3)
            o = jnp.concatenate([ot_scr[t].T for t in range(NQB)], axis=0)
            h = x_ref[...].astype(jnp.float32) + _dot(o, wo_v[...])
            h_scr[fslot] = h
            st["h"] = h

        def f_ln2():
            y_scr[fslot] = _layernorm(_layernorm(st.pop("h"))).astype(jnp.bfloat16)

        return dict(ln1=f_ln1, q=f_q, k=f_k, v=f_v, qk=qk, sm=sm, pv=pv, wo=f_wo, ln2=f_ln2)

    nst = NQB * HG

    def mm1(c):
        def run():
            cs = slice(FC * c, FC * (c + 1))
            hh = _dot(y_scr[bslot], w1_v[:, cs]) + b1_ref[:, cs].astype(jnp.float32)
            hh_scr[:, cs] = _gelu_tanh(hh).astype(jnp.bfloat16)
        return run

    def mm2(n):
        def run():
            ns = slice(NC * n, NC * (n + 1))
            out = (h_scr[bslot, :, ns] + b2_ref[:, ns].astype(jnp.float32)
                   + _dot(hh_scr[...], w2_v[:, ns]))
            o_ref[:, ns] = out.astype(o_ref.dtype)
        return run

    back = [mm1(c) for c in range(NF)] + [mm2(n) for n in range(NN)]
    bcost = [FC * TM * D // 65536] * NF + [NC * TM * F // 65536] * NN

    @pl.when(step == 0)
    def _():
        for c in copies[:4]:
            c.start()
        for c in copies[4:]:
            c.start(priority=1)
        k_scr[:, 0:W, :] = jnp.zeros((HG, W, 128), jnp.bfloat16)
        vt_scr[0:2] = jnp.zeros((2, D, 128), jnp.bfloat16)

    @pl.when(step < SKEW)
    def _():
        f = make_front(True)
        f["ln1"](); f["q"](); f["k"](); f["v"]()
        for s in range(nst + 2):
            if s < nst:
                f["qk"](s)
            if 0 <= s - 1 < nst:
                f["sm"](s - 1)
            if 0 <= s - 2 < nst:
                f["pv"](s - 2)
        f["wo"](); f["ln2"]()

    @pl.when(step == SKEW)
    def _():
        copies[4].wait()
        copies[5].wait()

    @pl.when(jnp.logical_and(step >= SKEW, step < NS))
    def _():
        f = make_front(False)
        bq = list(zip(back, bcost))

        def run_back(budget):
            used = 0
            while bq and used < budget:
                p, c = bq.pop(0)
                p()
                used += c

        total_b = sum(bcost)
        if ORDER == "A":
            run_back(1)
            f["ln1"](); f["q"](); f["k"](); f["v"]()
            tail = 2 * NC * TM * F // 65536
            per = (total_b - bcost[0] - tail) / nst
            done = 0
            for s in range(nst):
                f["qk"](s)
                before = sum(c for _, c in bq)
                run_back(per * (s + 1) - done)
                done += before - sum(c for _, c in bq)
                f["sm"](s)
                f["pv"](s)
            f["wo"]()
            run_back(1)
            f["ln2"]()
            run_back(1 << 30)
        elif ORDER == "B":
            run_back(1)
            f["ln1"](); f["q"](); f["k"](); f["v"]()
            tail = 2 * NC * TM * F // 65536
            per = (total_b - bcost[0] - tail) / (nst + 2)
            done = 0
            for s in range(nst + 2):
                if s < nst:
                    f["qk"](s)
                before = sum(c for _, c in bq)
                run_back(per * (s + 1) - done)
                done += before - sum(c for _, c in bq)
                if 0 <= s - 1 < nst:
                    f["sm"](s - 1)
                if 0 <= s - 2 < nst:
                    f["pv"](s - 2)
            f["wo"]()
            run_back(1)
            f["ln2"]()
            run_back(1 << 30)
        elif ORDER == "C":
            run_back(1)
            f["ln1"](); f["q"](); f["k"](); f["v"]()
            tail = 2 * NC * TM * F // 65536
            per = (total_b - bcost[0] - tail) / nst
            done = 0
            for s in range(nst):
                f["qk"](s)
                f["sm"](s)
                before = sum(c for _, c in bq)
                run_back(per * (s + 1) - done)
                done += before - sum(c for _, c in bq)
                f["pv"](s)
            f["wo"]()
            run_back(1)
            f["ln2"]()
            run_back(1 << 30)

        elif ORDER == "D":
            run_back(1)
            f["ln1"](); f["q"](); f["k"](); f["v"]()
            tail = NC * TM * F // 65536
            per = (total_b - bcost[0] - tail) / (2 * nst)
            done = 0
            def rb(k):
                nonlocal done
                before = sum(c for _, c in bq)
                run_back(per * k - done)
                done += before - sum(c for _, c in bq)
            for s in range(nst):
                f["qk"](s)
                rb(2 * s + 1)
                f["sm"](s)
                f["pv"](s)
                rb(2 * s + 2)
            f["wo"]()
            run_back(1)
            f["ln2"]()
            run_back(1 << 30)

        elif ORDER == "E":
            run_back(1)
            f["ln1"](); f["q"](); f["k"](); f["v"]()
            tail = NC * TM * F // 65536
            per = (total_b - bcost[0] - tail) / (2 * nst)
            done = 0
            def rb(k):
                nonlocal done
                before = sum(c for _, c in bq)
                run_back(per * k - done)
                done += before - sum(c for _, c in bq)
            for s in range(nst):
                f["qk"](s)
                f["sm"](s)
                rb(2 * s + 1)
                f["pv"](s)
                rb(2 * s + 2)
            f["wo"]()
            run_back(1)
            f["ln2"]()
            run_back(1 << 30)
        elif ORDER == "F":
            run_back(1)
            f["ln1"](); f["q"](); f["k"](); f["v"]()
            tail = NC * TM * F // 65536
            per = (total_b - bcost[0] - tail) / (2 * nst)
            done = 0
            def rb(k):
                nonlocal done
                before = sum(c for _, c in bq)
                run_back(per * k - done)
                done += before - sum(c for _, c in bq)
            for s in range(nst + 1):
                if s < nst: f["qk"](s)
                if s < nst: rb(2 * s + 1)
                if s >= 1: f["pv"](s - 1)
                if s < nst: f["sm"](s)
                if s < nst: rb(2 * s + 2)
            f["wo"]()
            run_back(1)
            f["ln2"]()
            run_back(1 << 30)

    @pl.when(step >= NS)
    def _():
        for p in back:
            p()


@jax.jit
def pallas_sequential_preLN__sliding_block__mixer_channel_mlp__prompt_kernel(
    A_x: jax.Array,
    A_wqkv: jax.Array,
    A_wo: jax.Array,
    B_x: jax.Array,
    B_w1: jax.Array,
    B_b1: jax.Array,
    B_w2: jax.Array,
    B_b2: jax.Array,
):
    x = A_x.reshape(S, D)
    b1 = B_b1.reshape(1, F)
    b2 = B_b2.reshape(1, D)

    grid_spec = pltpu.PrefetchScalarGridSpec(
        num_scalar_prefetch=0,
        grid=(NS + SKEW,),
        in_specs=[
            pl.BlockSpec((TM, D), lambda i: (jnp.minimum(i, NS - 1), 0)),
            pl.BlockSpec(memory_space=pl.ANY),
            pl.BlockSpec(memory_space=pl.ANY),
            pl.BlockSpec(memory_space=pl.ANY),
            pl.BlockSpec((1, F), lambda i: (0, 0)),
            pl.BlockSpec(memory_space=pl.ANY),
            pl.BlockSpec((1, D), lambda i: (0, 0)),
        ],
        out_specs=pl.BlockSpec((TM, D), lambda i: (jnp.maximum(i - SKEW, 0), 0)),
        scratch_shapes=[
            pltpu.VMEM((D, 3 * D), jnp.bfloat16),
            pltpu.VMEM((D, D), jnp.bfloat16),
            pltpu.VMEM((D, F), jnp.bfloat16),
            pltpu.VMEM((F, D), jnp.bfloat16),
            pltpu.VMEM((HG, S + W, 128), jnp.bfloat16),
            pltpu.VMEM((S // QB + 2, D, 128), jnp.bfloat16),
            pltpu.VMEM((HG, 4, TM, 128), jnp.bfloat16),
            pltpu.VMEM((NQB, D, 128), jnp.bfloat16),
            pltpu.VMEM((NSLOT, TM, D), jnp.bfloat16),
            pltpu.VMEM((NSLOT, TM, D), jnp.float32),
            pltpu.VMEM((TM, F), jnp.bfloat16),
            pltpu.VMEM((2, 2 * QB, 4 * QB), jnp.float32),
            pltpu.VMEM((2, 3 * QB, 4 * QB), jnp.bfloat16),
            pltpu.SemaphoreType.DMA((6,)),
        ],
    )
    out = pl.pallas_call(
        _kernel,
        grid_spec=grid_spec,
        out_shape=jax.ShapeDtypeStruct((S, D), jnp.bfloat16),
        compiler_params=pltpu.CompilerParams(
            dimension_semantics=("arbitrary",),
            vmem_limit_bytes=100 * 1024 * 1024,
        ),
    )(x, A_wqkv, A_wo, B_w1, b1, B_w2, b2)
    return out.reshape(1, S, D)
```

```python
import jax
import jax.numpy as jnp
import jax.experimental.pallas as pl
import jax.experimental.pallas.tpu as pltpu

S = 2048
D = 1024
DH = 32
W = 256
F = 3584
HG = 8
TM = 128
NS = S // TM
SKEW = 3
NSLOT = SKEW + 1
EPS = 1e-5
NEG = -1e30
QSCALE = (DH ** -0.5) * 1.4426950408889634
FC = 256
NC = 128
NF = F // FC
NN = D // NC
QH = D // 2


def _layernorm(x):
    m = jnp.mean(x, axis=-1, keepdims=True)
    xc = x - m
    v = jnp.mean(xc * xc, axis=-1, keepdims=True)
    return xc * jax.lax.rsqrt(v + EPS)


def _gelu_tanh(x):
    c = 0.7978845608028654
    inner = x * (c + (c * 0.044715) * (x * x))
    hx = 0.5 * x
    return hx + hx * jnp.tanh(inner)


def _dot(a, b):
    return jnp.dot(a, b, preferred_element_type=jnp.float32)


def _kernel(x_hbm, wqkv_hbm, wo_hbm, w1_hbm, b1_hbm, w2_hbm, b2_hbm, o_ref,
            wqkv_v, wo_v, w1_v, w2_v, x_scr, xn_scr, k_scr, vt_scr, qm_scr, ot_scr,
            y_scr, h_scr, hh_scr, s_scr, b1_ref, b2_ref, align_pad, sems):
    step = pl.program_id(0)
    fslot = step % NSLOT
    bslot = (step + 1) % NSLOT

    def wqkv_copy(lo, hi, sem):
        return pltpu.make_async_copy(wqkv_hbm.at[:, lo:hi], wqkv_v.at[:, lo:hi], sems.at[sem])

    def x_copy(blk, sem):
        row0 = pl.multiple_of(blk * TM, TM)
        return pltpu.make_async_copy(x_hbm.at[pl.ds(row0, TM), :], x_scr.at[blk % NSLOT], sems.at[sem])

    cp_b1 = pltpu.make_async_copy(b1_hbm, b1_ref, sems.at[11])
    cp_b2 = pltpu.make_async_copy(b2_hbm, b2_ref, sems.at[12])
    cp_q0 = wqkv_copy(0, QH, 3)
    cp_q1 = wqkv_copy(QH, D, 4)
    cp_k = wqkv_copy(D, 2 * D, 5)
    cp_v = wqkv_copy(2 * D, 3 * D, 6)
    cp_wo = pltpu.make_async_copy(wo_hbm, wo_v, sems.at[7])
    cp_w1 = pltpu.make_async_copy(w1_hbm, w1_v, sems.at[9])
    cp_w2 = pltpu.make_async_copy(w2_hbm, w2_v, sems.at[10])

    def proj_q(xn, qslot, lo, hi):
        q = _dot(xn, wqkv_v[:, lo:hi]) * QSCALE
        lane = jax.lax.broadcasted_iota(jnp.int32, (TM, 128), 1)
        for j in range((hi - lo) // 128):
            qh = q[:, 128 * j:128 * (j + 1)]
            for g in range(4):
                keep = (lane >= DH * g) & (lane < DH * (g + 1))
                qm_scr[qslot, lo // 128 + j, g] = jnp.where(keep, qh, 0.0).astype(jnp.bfloat16)

    def proj_k(xn, blk):
        row0 = pl.multiple_of(blk * TM + W, TM)
        k = _dot(xn, wqkv_v[:, D:2 * D]).astype(jnp.bfloat16)
        for hg in range(HG):
            k_scr[hg, pl.ds(row0, TM), :] = k[:, 128 * hg:128 * (hg + 1)]

    def proj_v(xn, blk):
        v = _dot(xn, wqkv_v[:, 2 * D:3 * D])
        vt_scr[blk + 2] = v.T.astype(jnp.bfloat16)

    def make_attn(first):
        st = {}
        qslot = step if first else 0

        def qk(hg):
            q0 = pl.multiple_of(step * TM, TM)
            qm = qm_scr[qslot, hg].reshape(4 * TM, 128)
            kp = k_scr[hg, pl.ds(q0, 3 * TM), :]
            kp = jnp.concatenate(
                [c for r in range(8)
                 for c in (kp[16 * r:16 * r + 16], kp[2 * TM + 16 * r:2 * TM + 16 * r + 16])]
                + [kp[TM:2 * TM]], axis=0)
            st_ = jax.lax.dot_general(kp, qm, (((1,), (1,)), ((), ())),
                                      preferred_element_type=jnp.float32)
            lane = jax.lax.broadcasted_iota(jnp.int32, (TM, TM), 1)
            row = jax.lax.broadcasted_iota(jnp.int32, (TM, TM), 0)
            tri = jnp.concatenate([lane < row] * 4, axis=1)
            s0 = jnp.concatenate([st_[32 * r:32 * r + 16] for r in range(8)], axis=0)
            s2 = jnp.concatenate([st_[32 * r + 16:32 * r + 32] for r in range(8)], axis=0)
            s1 = st_[2 * TM:3 * TM]
            if first:
                s0 = jnp.where(step >= 2, s0, NEG)
                s1 = jnp.where(step >= 1, s1, NEG)
            sm_ = jnp.where(tri, s0, s2)
            m = jnp.maximum(jnp.max(sm_, axis=0, keepdims=True), jnp.max(s1, axis=0, keepdims=True))
            s_scr[hg % 2, 0:TM, :] = sm_
            s_scr[hg % 2, TM:2 * TM, :] = s1
            st["m", hg] = m

        def sm(hg):
            m = st.pop(("m", hg))
            pm = jnp.exp2(s_scr[hg % 2, 0:TM, :] - m)
            p1 = jnp.exp2(s_scr[hg % 2, TM:2 * TM, :] - m)
            l = jnp.sum(pm, axis=0, keepdims=True) + jnp.sum(p1, axis=0, keepdims=True)
            lane = jax.lax.broadcasted_iota(jnp.int32, (TM, TM), 1)
            row = jax.lax.broadcasted_iota(jnp.int32, (TM, TM), 0)
            tri = lane < row
            ps = []
            for g in range(4):
                gs = slice(TM * g, TM * (g + 1))
                ps.append((jnp.where(tri, pm[:, gs], 0.0).astype(jnp.bfloat16),
                           p1[:, gs].astype(jnp.bfloat16),
                           jnp.where(tri, 0.0, pm[:, gs]).astype(jnp.bfloat16)))
            st["p", hg] = (ps, l)

        def pv(hg):
            ps, l = st.pop(("p", hg))
            for g in range(4):
                r0 = (hg * 4 + g) * DH
                p0, p1, p2 = ps[g]
                ot = (_dot(vt_scr[step, r0:r0 + DH, :], p0)
                      + _dot(vt_scr[step + 1, r0:r0 + DH, :], p1)
                      + _dot(vt_scr[step + 2, r0:r0 + DH, :], p2))
                ot_scr[r0:r0 + DH, :] = (ot / l[:, TM * g:TM * (g + 1)]).astype(ot_scr.dtype)

        def wo():
            h = x_scr[fslot].astype(jnp.float32) + _dot(ot_scr[...].T, wo_v[...])
            h_scr[fslot] = h
            st["h"] = h

        def ln2():
            y_scr[fslot] = _layernorm(_layernorm(st.pop("h"))).astype(jnp.bfloat16)

        return qk, sm, pv, wo, ln2

    def mm1(c):
        def run():
            cs = slice(FC * c, FC * (c + 1))
            hh = _dot(y_scr[bslot], w1_v[:, cs]) + b1_ref[cs].astype(jnp.float32).reshape(1, FC)
            hh_scr[:, cs] = _gelu_tanh(hh).astype(jnp.bfloat16)
        return run

    def mm2(n):
        def run():
            ns = slice(NC * n, NC * (n + 1))
            out = (h_scr[bslot, :, ns] + b2_ref[ns].astype(jnp.float32).reshape(1, NC)
                   + _dot(hh_scr[...], w2_v[:, ns]))
            o_ref[:, ns] = out.astype(o_ref.dtype)
        return run

    back = [mm1(c) for c in range(NF)] + [mm2(n) for n in range(NN)]
    bcost = [FC * TM * D // 65536] * NF + [NC * TM * F // 65536] * NN

    def over_first_blocks(fn):
        def body(b, carry):
            fn(b)
            return carry
        jax.lax.fori_loop(0, SKEW, body, 0)

    def front_step():
        @pl.when(step == 0)
        def _():
            x_copy(0, 0).start()
            cp_q0.start()
            for b in range(1, SKEW):
                x_copy(b, b).start()
            for c in (cp_q1, cp_k, cp_v, cp_wo, cp_b1, cp_b2):
                c.start()
            for c in (cp_w1, cp_w2):
                c.start(priority=1)
            k_scr[:, 0:W, :] = jnp.zeros((HG, W, 128), jnp.bfloat16)
            vt_scr[0:2] = jnp.zeros((2, D, 128), jnp.bfloat16)
            for b in range(SKEW):
                x_copy(b, b).wait()
                xn_scr[b] = _layernorm(x_scr[b].astype(jnp.float32)).astype(jnp.bfloat16)
            cp_q0.wait()
            over_first_blocks(lambda b: proj_q(xn_scr[b], b, 0, QH))
            cp_q1.wait()
            over_first_blocks(lambda b: proj_q(xn_scr[b], b, QH, D))
            cp_k.wait()
            over_first_blocks(lambda b: proj_k(xn_scr[b], b))
            cp_v.wait()
            over_first_blocks(lambda b: proj_v(xn_scr[b], b))
            cp_wo.wait()

        @pl.when(step == SKEW - 1)
        def _():
            x_copy(SKEW, 8).start()

        qk, sm, pv, wo, ln2 = make_attn(True)
        for s in range(HG + 2):
            if s < HG:
                qk(s)
            if 0 <= s - 1 < HG:
                sm(s - 1)
            if 0 <= s - 2 < HG:
                pv(s - 2)
        wo()
        ln2()

    def mixed_step():
        @pl.when(step == SKEW)
        def _():
            cp_w1.wait()
            cp_w2.wait()
            cp_b1.wait()
            cp_b2.wait()

        x_copy(step, 8).wait()

        @pl.when(step + 1 < NS)
        def _():
            x_copy(step + 1, 8).start()

        qk, sm, pv, wo, ln2 = make_attn(False)
        bq = list(zip(back, bcost))
        done = [0]

        def run_back(upto):
            while bq and done[0] < upto:
                p, c = bq.pop(0)
                p()
                done[0] += c

        run_back(1)
        xn = _layernorm(x_scr[fslot].astype(jnp.float32)).astype(jnp.bfloat16)
        proj_q(xn, 0, 0, D)
        proj_k(xn, step)
        proj_v(xn, step)
        base = done[0]
        per = (sum(bcost) - base - bcost[-1]) / (2 * HG)
        for s in range(HG):
            qk(s)
            run_back(base + per * (2 * s + 1))
            sm(s)
            pv(s)
            run_back(base + per * (2 * s + 2))
        wo()
        run_back(done[0] + 1)
        ln2()
        run_back(1 << 30)

    def back_step():
        for p in back:
            p()

    def other_step():
        jax.lax.cond(step < SKEW, front_step, back_step)

    jax.lax.cond(jnp.logical_and(step >= SKEW, step < NS), mixed_step, other_step)


@jax.jit
def pallas_sequential_preLN__sliding_block__mixer_channel_mlp__prompt_kernel(
    A_x: jax.Array,
    A_wqkv: jax.Array,
    A_wo: jax.Array,
    B_x: jax.Array,
    B_w1: jax.Array,
    B_b1: jax.Array,
    B_w2: jax.Array,
    B_b2: jax.Array,
):
    x = A_x.reshape(S, D)

    grid_spec = pltpu.PrefetchScalarGridSpec(
        num_scalar_prefetch=0,
        grid=(NS + SKEW,),
        in_specs=[
            pl.BlockSpec(memory_space=pl.ANY),
            pl.BlockSpec(memory_space=pl.ANY),
            pl.BlockSpec(memory_space=pl.ANY),
            pl.BlockSpec(memory_space=pl.ANY),
            pl.BlockSpec(memory_space=pl.ANY),
            pl.BlockSpec(memory_space=pl.ANY),
            pl.BlockSpec(memory_space=pl.ANY),
        ],
        out_specs=pl.BlockSpec((TM, D), lambda i: (jnp.maximum(i - SKEW, 0), 0)),
        scratch_shapes=[
            pltpu.VMEM((D, 3 * D), jnp.bfloat16),
            pltpu.VMEM((D, D), jnp.bfloat16),
            pltpu.VMEM((D, F), jnp.bfloat16),
            pltpu.VMEM((F, D), jnp.bfloat16),
            pltpu.VMEM((NSLOT, TM, D), jnp.bfloat16),
            pltpu.VMEM((SKEW, TM, D), jnp.bfloat16),
            pltpu.VMEM((HG, S + W, 128), jnp.bfloat16),
            pltpu.VMEM((NS + 2, D, TM), jnp.bfloat16),
            pltpu.VMEM((SKEW, HG, 4, TM, 128), jnp.bfloat16),
            pltpu.VMEM((D, TM), jnp.bfloat16),
            pltpu.VMEM((NSLOT, TM, D), jnp.bfloat16),
            pltpu.VMEM((NSLOT, TM, D), jnp.float32),
            pltpu.VMEM((TM, F), jnp.bfloat16),
            pltpu.VMEM((2, 2 * TM, 4 * TM), jnp.float32),
            pltpu.VMEM((F,), jnp.bfloat16),
            pltpu.VMEM((D,), jnp.bfloat16),
            pltpu.VMEM((1536,), jnp.bfloat16),
            pltpu.SemaphoreType.DMA((13,)),
        ],
    )
    out = pl.pallas_call(
        _kernel,
        grid_spec=grid_spec,
        out_shape=jax.ShapeDtypeStruct((S, D), jnp.bfloat16),
        compiler_params=pltpu.CompilerParams(
            dimension_semantics=("arbitrary",),
            vmem_limit_bytes=100 * 1024 * 1024,
        ),
    )(x, A_wqkv, A_wo, B_w1, B_b1, B_w2, B_b2)
    return out.reshape(1, S, D)
```

```python
import jax
import jax.numpy as jnp
import jax.experimental.pallas as pl
import jax.experimental.pallas.tpu as pltpu

S = 2048
D = 1024
DH = 32
W = 256
F = 3584
HG = 8
TM = 128
HT = TM // 2
NS = S // TM
SKEW = 3
NSLOT = SKEW + 1
EPS = 1e-5
NEG = -1e30
QSCALE = (DH ** -0.5) * 1.4426950408889634
FC = 256
NC = 128
NF = F // FC
NN = D // NC
HEAD = 2
TAIL = 2
MIDW = 0.7
QH = D // 2


def _layernorm(x):
    m = jnp.mean(x, axis=-1, keepdims=True)
    xc = x - m
    v = jnp.mean(xc * xc, axis=-1, keepdims=True)
    return xc * jax.lax.rsqrt(v + EPS)


def _gelu_tanh(x):
    c = 0.7978845608028654
    inner = x * (c + (c * 0.044715) * (x * x))
    hx = 0.5 * x
    return hx + hx * jnp.tanh(inner)


def _dot(a, b):
    return jnp.dot(a, b, preferred_element_type=jnp.float32)


def _kernel(x_hbm, wqkv_hbm, wo_hbm, w1_hbm, b1_hbm, w2_hbm, b2_hbm, o_ref,
            wqkv_v, wo_v, w1_v, w2_v, x_scr, xn_scr, k_scr, vt_scr, qm_scr, ot_scr,
            y_scr, h_scr, hh_scr, s_scr, b1_ref, b2_ref, align_pad, sems):
    step = pl.program_id(0)
    fslot = step % NSLOT
    bslot = (step + 1) % NSLOT

    def wqkv_copy(lo, hi, sem):
        return pltpu.make_async_copy(wqkv_hbm.at[:, lo:hi], wqkv_v.at[:, lo:hi], sems.at[sem])

    def x_copy(blk, sem):
        row0 = pl.multiple_of(blk * TM, TM)
        return pltpu.make_async_copy(x_hbm.at[pl.ds(row0, TM), :], x_scr.at[blk % NSLOT], sems.at[sem])

    cp_b1 = pltpu.make_async_copy(b1_hbm, b1_ref, sems.at[11])
    cp_b2 = pltpu.make_async_copy(b2_hbm, b2_ref, sems.at[12])
    cp_q0 = wqkv_copy(0, QH, 3)
    cp_q1 = wqkv_copy(QH, D, 4)
    cp_k = wqkv_copy(D, 2 * D, 5)
    cp_v = wqkv_copy(2 * D, 3 * D, 6)
    cp_wo = pltpu.make_async_copy(wo_hbm, wo_v, sems.at[7])
    cp_w1 = pltpu.make_async_copy(w1_hbm, w1_v, sems.at[9])
    cp_w2 = pltpu.make_async_copy(w2_hbm, w2_v, sems.at[10])

    def proj_q(xn, qslot, lo, hi):
        q = _dot(xn, wqkv_v[:, lo:hi]) * QSCALE
        lane = jax.lax.broadcasted_iota(jnp.int32, (TM, 128), 1)
        for j in range((hi - lo) // 128):
            qh = q[:, 128 * j:128 * (j + 1)]
            for g in range(4):
                keep = (lane >= DH * g) & (lane < DH * (g + 1))
                qm_scr[qslot, lo // 128 + j, g] = jnp.where(keep, qh, 0.0).astype(jnp.bfloat16)

    def proj_k(xn, blk):
        row0 = pl.multiple_of(blk * TM + W, TM)
        k = _dot(xn, wqkv_v[:, D:2 * D]).astype(jnp.bfloat16)
        for hg in range(HG):
            k_scr[hg, pl.ds(row0, TM), :] = k[:, 128 * hg:128 * (hg + 1)]

    def proj_v(xn, blk):
        v = _dot(xn, wqkv_v[:, 2 * D:3 * D])
        vt_scr[blk + 2] = v.T.astype(jnp.bfloat16)

    def make_attn(first):
        st = {}
        qslot = step if first else 0

        def qk(hg):
            q0 = pl.multiple_of(step * TM, TM)
            nt = (((1,), (1,)), ((), ()))
            qm = qm_scr[qslot, hg]
            kp = k_scr[hg, pl.ds(q0, 3 * TM), :]
            hi = jax.lax.broadcasted_iota(jnp.int32, (HT, 128), 1) >= 64
            la = jnp.where(hi, kp[2 * TM + HT:3 * TM], kp[0:HT])
            lb = jnp.where(hi, kp[0:HT], kp[2 * TM + HT:3 * TM])
            xa = jnp.concatenate([qm[0, 0:HT], qm[2, HT:TM], qm[1, 0:HT], qm[3, HT:TM]], axis=0)
            xb = jnp.concatenate([qm[2, 0:HT], qm[0, HT:TM], qm[3, 0:HT], qm[1, HT:TM]], axis=0)
            ea = jax.lax.dot_general(la, xa, nt, preferred_element_type=jnp.float32)
            eb = jax.lax.dot_general(lb, xb, nt, preferred_element_type=jnp.float32)
            kmain = jnp.concatenate([kp[2 * TM:2 * TM + HT], kp[HT:TM], kp[TM:2 * TM]], axis=0)
            st_ = jax.lax.dot_general(kmain, qm.reshape(4 * TM, 128), nt,
                                      preferred_element_type=jnp.float32)
            lane = jax.lax.broadcasted_iota(jnp.int32, (TM, TM), 1)
            row = jax.lax.broadcasted_iota(jnp.int32, (TM, TM), 0)
            tri = jnp.concatenate([lane < row] * 4, axis=1)
            s0 = jnp.concatenate([ea, eb], axis=1)
            s0 = jnp.concatenate([s0, st_[HT:TM]], axis=0)
            s2 = jnp.concatenate([eb, ea], axis=1)
            s2 = jnp.concatenate([st_[0:HT], s2], axis=0)
            s1 = st_[TM:2 * TM]
            if first:
                s0 = jnp.where(step >= 2, s0, NEG)
                s1 = jnp.where(step >= 1, s1, NEG)
            sm_ = jnp.where(tri, s0, s2)
            m = jnp.maximum(jnp.max(sm_, axis=0, keepdims=True), jnp.max(s1, axis=0, keepdims=True))
            s_scr[hg % 2, 0:TM, :] = sm_
            s_scr[hg % 2, TM:2 * TM, :] = s1
            st["m", hg] = m

        def sm(hg):
            m = st.pop(("m", hg))
            pm = jnp.exp2(s_scr[hg % 2, 0:TM, :] - m)
            p1 = jnp.exp2(s_scr[hg % 2, TM:2 * TM, :] - m)
            l = jnp.sum(pm, axis=0, keepdims=True) + jnp.sum(p1, axis=0, keepdims=True)
            lane = jax.lax.broadcasted_iota(jnp.int32, (TM, TM), 1)
            row = jax.lax.broadcasted_iota(jnp.int32, (TM, TM), 0)
            tri = lane < row
            ps = []
            for g in range(4):
                gs = slice(TM * g, TM * (g + 1))
                ps.append((jnp.where(tri, pm[:, gs], 0.0).astype(jnp.bfloat16),
                           p1[:, gs].astype(jnp.bfloat16),
                           jnp.where(tri, 0.0, pm[:, gs]).astype(jnp.bfloat16)))
            st["p", hg] = (ps, l)

        def pv(hg):
            ps, l = st.pop(("p", hg))
            for g in range(4):
                r0 = (hg * 4 + g) * DH
                p0, p1, p2 = ps[g]
                ot = (_dot(vt_scr[step, r0:r0 + DH, :], p0)
                      + _dot(vt_scr[step + 1, r0:r0 + DH, :], p1)
                      + _dot(vt_scr[step + 2, r0:r0 + DH, :], p2))
                ot_scr[r0:r0 + DH, :] = (ot / l[:, TM * g:TM * (g + 1)]).astype(ot_scr.dtype)

        def wo():
            h = x_scr[fslot].astype(jnp.float32) + _dot(ot_scr[...].T, wo_v[...])
            h_scr[fslot] = h
            st["h"] = h

        def ln2():
            y_scr[fslot] = _layernorm(_layernorm(st.pop("h"))).astype(jnp.bfloat16)

        return qk, sm, pv, wo, ln2

    def mm1(c):
        def run():
            cs = slice(FC * c, FC * (c + 1))
            hh = _dot(y_scr[bslot], w1_v[:, cs]) + b1_ref[cs].astype(jnp.float32).reshape(1, FC)
            hh_scr[:, cs] = _gelu_tanh(hh).astype(jnp.bfloat16)
        return run

    def mm2(n):
        def run():
            ns = slice(NC * n, NC * (n + 1))
            out = (h_scr[bslot, :, ns] + b2_ref[ns].astype(jnp.float32).reshape(1, NC)
                   + _dot(hh_scr[...], w2_v[:, ns]))
            o_ref[:, ns] = out.astype(o_ref.dtype)
        return run

    back = [mm1(c) for c in range(NF)] + [mm2(n) for n in range(NN)]
    bcost = [FC * TM * D // 65536] * NF + [NC * TM * F // 65536] * NN

    def over_first_blocks(fn):
        def body(b, carry):
            fn(b)
            return carry
        jax.lax.fori_loop(0, SKEW, body, 0)

    def front_step():
        @pl.when(step == 0)
        def _():
            x_copy(0, 0).start()
            cp_q0.start()
            for b in range(1, SKEW):
                x_copy(b, b).start()
            for c in (cp_q1, cp_k, cp_v, cp_wo, cp_b1, cp_b2):
                c.start()
            for c in (cp_w1, cp_w2):
                c.start(priority=1)
            k_scr[:, 0:W, :] = jnp.zeros((HG, W, 128), jnp.bfloat16)
            vt_scr[0:2] = jnp.zeros((2, D, 128), jnp.bfloat16)
            for b in range(SKEW):
                x_copy(b, b).wait()
                xn_scr[b] = _layernorm(x_scr[b].astype(jnp.float32)).astype(jnp.bfloat16)
            cp_q0.wait()
            over_first_blocks(lambda b: proj_q(xn_scr[b], b, 0, QH))
            cp_q1.wait()
            over_first_blocks(lambda b: proj_q(xn_scr[b], b, QH, D))
            cp_k.wait()
            over_first_blocks(lambda b: proj_k(xn_scr[b], b))
            cp_v.wait()
            over_first_blocks(lambda b: proj_v(xn_scr[b], b))
            cp_wo.wait()

        @pl.when(step == SKEW - 1)
        def _():
            x_copy(SKEW, 8).start()

        qk, sm, pv, wo, ln2 = make_attn(True)
        for s in range(HG + 2):
            if s < HG:
                qk(s)
            if 0 <= s - 1 < HG:
                sm(s - 1)
            if 0 <= s - 2 < HG:
                pv(s - 2)
        wo()
        ln2()

    def mixed_step():
        @pl.when(step == SKEW)
        def _():
            cp_w1.wait()
            cp_w2.wait()
            cp_b1.wait()
            cp_b2.wait()

        x_copy(step, 8).wait()

        @pl.when(step + 1 < NS)
        def _():
            x_copy(step + 1, 8).start()

        qk, sm, pv, wo, ln2 = make_attn(False)
        bq = list(zip(back, bcost))
        done = [0]

        def run_back(upto):
            while bq and done[0] < upto:
                p, c = bq.pop(0)
                p()
                done[0] += c

        run_back(HEAD * bcost[0])
        xn = _layernorm(x_scr[fslot].astype(jnp.float32)).astype(jnp.bfloat16)
        proj_q(xn, 0, 0, D)
        proj_k(xn, step)
        proj_v(xn, step)
        base = done[0]
        per = (sum(bcost) - base - TAIL * bcost[-1]) / HG
        for s in range(HG):
            qk(s)
            run_back(base + per * (s + MIDW))
            sm(s)
            pv(s)
            run_back(base + per * (s + 1))
        wo()
        run_back(done[0] + 1)
        ln2()
        run_back(1 << 30)

    def back_step():
        for p in back:
            p()

    def other_step():
        jax.lax.cond(step < SKEW, front_step, back_step)

    jax.lax.cond(jnp.logical_and(step >= SKEW, step < NS), mixed_step, other_step)


@jax.jit
def pallas_sequential_preLN__sliding_block__mixer_channel_mlp__prompt_kernel(
    A_x: jax.Array,
    A_wqkv: jax.Array,
    A_wo: jax.Array,
    B_x: jax.Array,
    B_w1: jax.Array,
    B_b1: jax.Array,
    B_w2: jax.Array,
    B_b2: jax.Array,
):
    x = A_x.reshape(S, D)

    grid_spec = pltpu.PrefetchScalarGridSpec(
        num_scalar_prefetch=0,
        grid=(NS + SKEW,),
        in_specs=[
            pl.BlockSpec(memory_space=pl.ANY),
            pl.BlockSpec(memory_space=pl.ANY),
            pl.BlockSpec(memory_space=pl.ANY),
            pl.BlockSpec(memory_space=pl.ANY),
            pl.BlockSpec(memory_space=pl.ANY),
            pl.BlockSpec(memory_space=pl.ANY),
            pl.BlockSpec(memory_space=pl.ANY),
        ],
        out_specs=pl.BlockSpec((TM, D), lambda i: (jnp.maximum(i - SKEW, 0), 0)),
        scratch_shapes=[
            pltpu.VMEM((D, 3 * D), jnp.bfloat16),
            pltpu.VMEM((D, D), jnp.bfloat16),
            pltpu.VMEM((D, F), jnp.bfloat16),
            pltpu.VMEM((F, D), jnp.bfloat16),
            pltpu.VMEM((NSLOT, TM, D), jnp.bfloat16),
            pltpu.VMEM((SKEW, TM, D), jnp.bfloat16),
            pltpu.VMEM((HG, S + W, 128), jnp.bfloat16),
            pltpu.VMEM((NS + 2, D, TM), jnp.bfloat16),
            pltpu.VMEM((SKEW, HG, 4, TM, 128), jnp.bfloat16),
            pltpu.VMEM((D, TM), jnp.bfloat16),
            pltpu.VMEM((NSLOT, TM, D), jnp.bfloat16),
            pltpu.VMEM((NSLOT, TM, D), jnp.float32),
            pltpu.VMEM((TM, F), jnp.bfloat16),
            pltpu.VMEM((2, 2 * TM, 4 * TM), jnp.float32),
            pltpu.VMEM((F,), jnp.bfloat16),
            pltpu.VMEM((D,), jnp.bfloat16),
            pltpu.VMEM((1536,), jnp.bfloat16),
            pltpu.SemaphoreType.DMA((13,)),
        ],
    )
    out = pl.pallas_call(
        _kernel,
        grid_spec=grid_spec,
        out_shape=jax.ShapeDtypeStruct((S, D), jnp.bfloat16),
        compiler_params=pltpu.CompilerParams(
            dimension_semantics=("arbitrary",),
            vmem_limit_bytes=100 * 1024 * 1024,
            disable_bounds_checks=True,
        ),
    )(x, A_wqkv, A_wo, B_w1, B_b1, B_w2, B_b2)
    return out.reshape(1, S, D)
```

```python
import jax
import jax.numpy as jnp
import jax.experimental.pallas as pl
import jax.experimental.pallas.tpu as pltpu

S = 2048
D = 1024
DH = 32
W = 256
F = 3584
HG = 8
TM = 128
HT = TM // 2
NS = S // TM
SKEW = 3
NSLOT = SKEW + 1
EPS = 1e-5
NEG = -1e30
QSCALE = (DH ** -0.5) * 1.4426950408889634
FC = 256
NC = 128
NF = F // FC
NN = D // NC
HEAD = 2
TAIL = 2
MIDW = 0.7
QH = D // 2


def _layernorm(x):
    m = jnp.mean(x, axis=-1, keepdims=True)
    xc = x - m
    v = jnp.mean(xc * xc, axis=-1, keepdims=True)
    return xc * jax.lax.rsqrt(v + EPS)


def _gelu_tanh(x):
    c = 0.7978845608028654
    inner = x * (c + (c * 0.044715) * (x * x))
    hx = 0.5 * x
    return hx + hx * jnp.tanh(inner)


def _dot(a, b):
    return jnp.dot(a, b, preferred_element_type=jnp.float32)


def _kernel(x_hbm, wqkv_hbm, wo_hbm, w1_hbm, b1_hbm, w2_hbm, b2_hbm, o_ref,
            wqkv_v, wo_v, w1_v, w2_v, x_scr, xn_scr, k_scr, vt_scr, qm_scr, ot_scr,
            y_scr, h_scr, hh_scr, s_scr, b1_ref, b2_ref, align_pad, sems):
    step = pl.program_id(0)
    fslot = step % NSLOT
    bslot = (step + 1) % NSLOT

    def wqkv_copy(lo, hi, sem):
        return pltpu.make_async_copy(wqkv_hbm.at[:, lo:hi], wqkv_v.at[:, lo:hi], sems.at[sem])

    def x_copy(blk, sem):
        row0 = pl.multiple_of(blk * TM, TM)
        return pltpu.make_async_copy(x_hbm.at[pl.ds(row0, TM), :], x_scr.at[blk % NSLOT], sems.at[sem])

    cp_b1 = pltpu.make_async_copy(b1_hbm, b1_ref, sems.at[11])
    cp_b2 = pltpu.make_async_copy(b2_hbm, b2_ref, sems.at[12])
    cp_q0 = wqkv_copy(0, QH, 3)
    cp_q1 = wqkv_copy(QH, D, 4)
    cp_k = wqkv_copy(D, 2 * D, 5)
    cp_v = wqkv_copy(2 * D, 3 * D, 6)
    cp_wo = pltpu.make_async_copy(wo_hbm, wo_v, sems.at[7])
    cp_w1 = pltpu.make_async_copy(w1_hbm, w1_v, sems.at[9])
    cp_w2 = pltpu.make_async_copy(w2_hbm, w2_v, sems.at[10])

    def proj_q(xn, qslot, lo, hi):
        q = _dot(xn, wqkv_v[:, lo:hi]) * QSCALE
        lane = jax.lax.broadcasted_iota(jnp.int32, (TM, 128), 1)
        for j in range((hi - lo) // 128):
            qh = q[:, 128 * j:128 * (j + 1)]
            for g in range(4):
                keep = (lane >= DH * g) & (lane < DH * (g + 1))
                qm_scr[qslot, lo // 128 + j, g] = jnp.where(keep, qh, 0.0).astype(jnp.bfloat16)

    def proj_k(xn, blk):
        row0 = pl.multiple_of(blk * TM + W, TM)
        k = _dot(xn, wqkv_v[:, D:2 * D]).astype(jnp.bfloat16)
        for hg in range(HG):
            k_scr[hg, pl.ds(row0, TM), :] = k[:, 128 * hg:128 * (hg + 1)]

    def proj_v(xn, blk):
        v = _dot(xn, wqkv_v[:, 2 * D:3 * D])
        vt_scr[blk + 2] = v.T.astype(jnp.bfloat16)

    def make_attn(first):
        st = {}
        qslot = step if first else 0

        def qk(hg):
            q0 = pl.multiple_of(step * TM, TM)
            nt = (((1,), (1,)), ((), ()))
            qm = qm_scr[qslot, hg]
            kp = k_scr[hg, pl.ds(q0, 3 * TM), :]
            hi = jax.lax.broadcasted_iota(jnp.int32, (HT, 128), 1) >= 64
            la = jnp.where(hi, kp[2 * TM + HT:3 * TM], kp[0:HT])
            lb = jnp.where(hi, kp[0:HT], kp[2 * TM + HT:3 * TM])
            xa = jnp.concatenate([qm[0, 0:HT], qm[2, HT:TM], qm[1, 0:HT], qm[3, HT:TM]], axis=0)
            xb = jnp.concatenate([qm[2, 0:HT], qm[0, HT:TM], qm[3, 0:HT], qm[1, HT:TM]], axis=0)
            ea = jax.lax.dot_general(la, xa, nt, preferred_element_type=jnp.float32)
            eb = jax.lax.dot_general(lb, xb, nt, preferred_element_type=jnp.float32)
            kmain = jnp.concatenate([kp[2 * TM:2 * TM + HT], kp[HT:TM], kp[TM:2 * TM]], axis=0)
            st_ = jax.lax.dot_general(kmain, qm.reshape(4 * TM, 128), nt,
                                      preferred_element_type=jnp.float32)
            lane = jax.lax.broadcasted_iota(jnp.int32, (TM, TM), 1)
            row = jax.lax.broadcasted_iota(jnp.int32, (TM, TM), 0)
            tri = jnp.concatenate([lane < row] * 4, axis=1)
            s0 = jnp.concatenate([ea, eb], axis=1)
            s0 = jnp.concatenate([s0, st_[HT:TM]], axis=0)
            s2 = jnp.concatenate([eb, ea], axis=1)
            s2 = jnp.concatenate([st_[0:HT], s2], axis=0)
            s1 = st_[TM:2 * TM]
            if first:
                s0 = jnp.where(step >= 2, s0, NEG)
                s1 = jnp.where(step >= 1, s1, NEG)
            sm_ = jnp.where(tri, s0, s2)
            m = jnp.maximum(jnp.max(sm_, axis=0, keepdims=True), jnp.max(s1, axis=0, keepdims=True))
            s_scr[hg % 2, 0:TM, :] = sm_
            s_scr[hg % 2, TM:2 * TM, :] = s1
            st["m", hg] = m

        def sm(hg):
            m = st.pop(("m", hg))
            pm = jnp.exp2(s_scr[hg % 2, 0:TM, :] - m)
            p1 = jnp.exp2(s_scr[hg % 2, TM:2 * TM, :] - m)
            l = jnp.sum(pm, axis=0, keepdims=True) + jnp.sum(p1, axis=0, keepdims=True)
            lane = jax.lax.broadcasted_iota(jnp.int32, (TM, TM), 1)
            row = jax.lax.broadcasted_iota(jnp.int32, (TM, TM), 0)
            tri = lane < row
            ps = []
            for g in range(4):
                gs = slice(TM * g, TM * (g + 1))
                ps.append((jnp.where(tri, pm[:, gs], 0.0).astype(jnp.bfloat16),
                           p1[:, gs].astype(jnp.bfloat16),
                           jnp.where(tri, 0.0, pm[:, gs]).astype(jnp.bfloat16)))
            st["p", hg] = (ps, l)

        def pv(hg):
            ps, l = st.pop(("p", hg))
            for g in range(4):
                r0 = (hg * 4 + g) * DH
                p0, p1, p2 = ps[g]
                ot = (_dot(vt_scr[step, r0:r0 + DH, :], p0)
                      + _dot(vt_scr[step + 1, r0:r0 + DH, :], p1)
                      + _dot(vt_scr[step + 2, r0:r0 + DH, :], p2))
                ot_scr[r0:r0 + DH, :] = (ot / l[:, TM * g:TM * (g + 1)]).astype(ot_scr.dtype)

        def wo():
            h = x_scr[fslot].astype(jnp.float32) + _dot(ot_scr[...].T, wo_v[...])
            h_scr[fslot] = h
            st["h"] = h

        def ln2():
            y_scr[fslot] = _layernorm(_layernorm(st.pop("h"))).astype(jnp.bfloat16)

        return qk, sm, pv, wo, ln2

    def mm1(c):
        def run():
            cs = slice(FC * c, FC * (c + 1))
            hh = _dot(y_scr[bslot], w1_v[:, cs]) + b1_ref[cs].astype(jnp.float32).reshape(1, FC)
            hh_scr[:, cs] = _gelu_tanh(hh).astype(jnp.bfloat16)
        return run

    def mm2(n):
        def run():
            ns = slice(NC * n, NC * (n + 1))
            out = (h_scr[bslot, :, ns] + b2_ref[ns].astype(jnp.float32).reshape(1, NC)
                   + _dot(hh_scr[...], w2_v[:, ns]))
            o_ref[:, ns] = out.astype(o_ref.dtype)
        return run

    back = [mm1(c) for c in range(NF)] + [mm2(n) for n in range(NN)]
    bcost = [FC * TM * D // 65536] * NF + [NC * TM * F // 65536] * NN

    def over_first_blocks(fn):
        def body(b, carry):
            fn(b)
            return carry
        jax.lax.fori_loop(0, SKEW, body, 0)

    def front_step():
        @pl.when(step == 0)
        def _():
            x_copy(0, 13).start()
            cp_q0.start()
            for b in range(1, SKEW):
                x_copy(b, 13 + b).start()
            for c in (cp_q1, cp_k, cp_v, cp_wo, cp_b1, cp_b2):
                c.start()
            for c in (cp_w1, cp_w2):
                c.start(priority=1)
            k_scr[:, 0:W, :] = jnp.zeros((HG, W, 128), jnp.bfloat16)
            vt_scr[0:2] = jnp.zeros((2, D, 128), jnp.bfloat16)
            for b in range(SKEW):
                x_copy(b, 13 + b).wait()
                xn_scr[b] = _layernorm(x_scr[b].astype(jnp.float32)).astype(jnp.bfloat16)
            cp_q0.wait()
            over_first_blocks(lambda b: proj_q(xn_scr[b], b, 0, QH))
            cp_q1.wait()
            over_first_blocks(lambda b: proj_q(xn_scr[b], b, QH, D))
            cp_k.wait()
            over_first_blocks(lambda b: proj_k(xn_scr[b], b))
            cp_v.wait()
            over_first_blocks(lambda b: proj_v(xn_scr[b], b))
            cp_wo.wait()

        @pl.when(step == SKEW - 1)
        def _():
            x_copy(SKEW, 8).start()

        qk, sm, pv, wo, ln2 = make_attn(True)
        for s in range(HG + 2):
            if s < HG:
                qk(s)
            if 0 <= s - 1 < HG:
                sm(s - 1)
            if 0 <= s - 2 < HG:
                pv(s - 2)
        wo()
        ln2()

    def mixed_step():
        @pl.when(step == SKEW)
        def _():
            cp_w1.wait()
            cp_w2.wait()
            cp_b1.wait()
            cp_b2.wait()

        x_copy(step, 8).wait()

        @pl.when(step + 1 < NS)
        def _():
            x_copy(step + 1, 8).start()

        qk, sm, pv, wo, ln2 = make_attn(False)
        bq = list(zip(back, bcost))
        done = [0]

        def run_back(upto):
            while bq and done[0] < upto:
                p, c = bq.pop(0)
                p()
                done[0] += c

        run_back(HEAD * bcost[0])
        xn = _layernorm(x_scr[fslot].astype(jnp.float32)).astype(jnp.bfloat16)
        proj_q(xn, 0, 0, D)
        proj_k(xn, step)
        proj_v(xn, step)
        base = done[0]
        per = (sum(bcost) - base - TAIL * bcost[-1]) / HG
        for s in range(HG):
            qk(s)
            run_back(base + per * (s + MIDW))
            sm(s)
            pv(s)
            run_back(base + per * (s + 1))
        wo()
        run_back(done[0] + 1)
        ln2()
        run_back(1 << 30)

    def back_step():
        for p in back:
            p()

    def other_step():
        jax.lax.cond(step < SKEW, front_step, back_step)

    jax.lax.cond(jnp.logical_and(step >= SKEW, step < NS), mixed_step, other_step)


@jax.jit
def pallas_sequential_preLN__sliding_block__mixer_channel_mlp__prompt_kernel(
    A_x: jax.Array,
    A_wqkv: jax.Array,
    A_wo: jax.Array,
    B_x: jax.Array,
    B_w1: jax.Array,
    B_b1: jax.Array,
    B_w2: jax.Array,
    B_b2: jax.Array,
):
    x = A_x.reshape(S, D)

    grid_spec = pltpu.PrefetchScalarGridSpec(
        num_scalar_prefetch=0,
        grid=(NS + SKEW,),
        in_specs=[
            pl.BlockSpec(memory_space=pl.ANY),
            pl.BlockSpec(memory_space=pl.ANY),
            pl.BlockSpec(memory_space=pl.ANY),
            pl.BlockSpec(memory_space=pl.ANY),
            pl.BlockSpec(memory_space=pl.ANY),
            pl.BlockSpec(memory_space=pl.ANY),
            pl.BlockSpec(memory_space=pl.ANY),
        ],
        out_specs=pl.BlockSpec((TM, D), lambda i: (jnp.maximum(i - SKEW, 0), 0)),
        scratch_shapes=[
            pltpu.VMEM((D, 3 * D), jnp.bfloat16),
            pltpu.VMEM((D, D), jnp.bfloat16),
            pltpu.VMEM((D, F), jnp.bfloat16),
            pltpu.VMEM((F, D), jnp.bfloat16),
            pltpu.VMEM((NSLOT, TM, D), jnp.bfloat16),
            pltpu.VMEM((SKEW, TM, D), jnp.bfloat16),
            pltpu.VMEM((HG, S + W, 128), jnp.bfloat16),
            pltpu.VMEM((NS + 2, D, TM), jnp.bfloat16),
            pltpu.VMEM((SKEW, HG, 4, TM, 128), jnp.bfloat16),
            pltpu.VMEM((D, TM), jnp.bfloat16),
            pltpu.VMEM((NSLOT, TM, D), jnp.bfloat16),
            pltpu.VMEM((NSLOT, TM, D), jnp.float32),
            pltpu.VMEM((TM, F), jnp.bfloat16),
            pltpu.VMEM((2, 2 * TM, 4 * TM), jnp.float32),
            pltpu.VMEM((F,), jnp.bfloat16),
            pltpu.VMEM((D,), jnp.bfloat16),
            pltpu.VMEM((1536,), jnp.bfloat16),
            pltpu.SemaphoreType.DMA((13 + SKEW,)),
        ],
    )
    out = pl.pallas_call(
        _kernel,
        grid_spec=grid_spec,
        out_shape=jax.ShapeDtypeStruct((S, D), jnp.bfloat16),
        compiler_params=pltpu.CompilerParams(
            dimension_semantics=("arbitrary",),
            vmem_limit_bytes=100 * 1024 * 1024,
            disable_bounds_checks=True,
        ),
    )(x, A_wqkv, A_wo, B_w1, B_b1, B_w2, B_b2)
    return out.reshape(1, S, D)
```
